```python
import os as _os
_os.environ.setdefault("JAX_PLATFORMS", "cpu")
import jax
import jax.numpy as jnp

def _softmax(x, axis=-1):
    return jax.nn.softmax(x, axis=axis)
def _gelu(x):
    return jax.nn.gelu(x, approximate=True)
def _silu(x):
    return jax.nn.silu(x)
def _sigmoid(x):
    return jax.nn.sigmoid(x)
def _layernorm(x, axis=-1, eps=1e-5):
    m = jnp.mean(x, axis=axis, keepdims=True)
    v = jnp.var(x, axis=axis, keepdims=True)
    return (x - m) / jnp.sqrt(v + eps)
def _scatter_add(tgt, idx, src, axis=0):
    return tgt.at[idx].add(src)
def _segment_sum(src, seg, n):
    return jax.ops.segment_sum(src, seg, n)
class _Rng:
    def __init__(self, key):
        self._k = key
    def _next(self):
        self._k, sub = jax.random.split(self._k)
        return sub
    def normal(self, shape):
        return jax.random.normal(self._next(), shape, dtype=jnp.bfloat16)
    def randint(self, lo, hi, shape):
        return jax.random.randint(self._next(), shape, lo, hi, dtype=jnp.int32)
    def uniform(self, shape, lo=0.0, hi=1.0):
        return jax.random.uniform(self._next(), shape, jnp.bfloat16, lo, hi)
    def permutation(self, n):
        return jax.random.permutation(self._next(), n)


kernel_name = 'standalone__grn__sampling'

def setup_inputs():
    _rng = _Rng(jax.random.key(int.from_bytes(__import__("os").urandom(4), "little")))
    _w = (lambda a: (lambda t: t.astype(jnp.bfloat16) if jnp.issubdtype(t.dtype, jnp.floating) else t)(jnp.asarray(a)))
    B, S, D = 512, 32, 640
    return {
        "x": _w((lambda *s: _rng.normal(s) * 0.05)(B, S, D)),
        "g": _w((lambda *s: _rng.normal(s) * 0.1)(D) * 0.1),
        "b": _w((lambda *s: _rng.normal(s) * 0.1)(D) * 0.1),
    }

def reference(x, g, b):
    gx = jnp.sqrt((x * x).sum(axis=-2, keepdims=True))
    nx = gx / (gx.mean(axis=-1, keepdims=True) + 1e-6)
    return g * (x * nx) + b + x
```

```python
import jax
import jax.numpy as jnp
import jax.experimental.pallas as pl
import jax.experimental.pallas.tpu as pltpu


@jax.jit
def pallas_standalone__grn__sampling_kernel(
    x: jax.Array,
    g: jax.Array,
    b: jax.Array,
):
    B, S, D = x.shape
    TB = 32

    def kernel_function(x_ref, g_ref, b_ref, o_ref):
        xf = x_ref[...].astype(jnp.float32)
        gf = g_ref[...].astype(jnp.float32)
        bf = b_ref[...].astype(jnp.float32)
        gx = jnp.sqrt(jnp.sum(xf * xf, axis=1, keepdims=True))
        nx = gx / (jnp.mean(gx, axis=-1, keepdims=True) + 1e-6)
        scale = gf * nx + 1.0
        o_ref[...] = (xf * scale + bf).astype(o_ref.dtype)

    return pl.pallas_call(
        kernel_function,
        grid=(B // TB,),
        in_specs=[
            pl.BlockSpec((TB, S, D), lambda i: (i, 0, 0)),
            pl.BlockSpec((1, D), lambda i: (0, 0)),
            pl.BlockSpec((1, D), lambda i: (0, 0)),
        ],
        out_specs=pl.BlockSpec((TB, S, D), lambda i: (i, 0, 0)),
        out_shape=jax.ShapeDtypeStruct(x.shape, x.dtype),
        compiler_params=pltpu.CompilerParams(dimension_semantics=("parallel",)),
    )(x, g.reshape(1, D), b.reshape(1, D))
```

```python
import jax
import jax.numpy as jnp
import jax.experimental.pallas as pl
import jax.experimental.pallas.tpu as pltpu

_K = 8
_TB = 32
_TAIL = 8
_G = 8
_SPLIT = 2


@jax.jit
def pallas_standalone__grn__sampling_kernel(
    x: jax.Array,
    g: jax.Array,
    b: jax.Array,
):
    B, S, D = x.shape
    K, TB, TAIL, G = _K, _TB, _TAIL, _G
    M = B // K
    CPS = M // TB
    NCU = B // TB - 1
    SP = S // _SPLIT

    def kernel_function(x_hbm, g_hbm, b_hbm, o_hbm,
                        xbuf, obuf, gbuf, bbuf, sc_ref, rsem, wsem, psem):
        def read(i, s, off, n):
            return pltpu.make_async_copy(
                x_hbm.at[s, pl.ds(off, n)], xbuf.at[s, pl.ds(off, n)], rsem.at[i])

        gcp = pltpu.make_async_copy(g_hbm, gbuf, psem.at[0])
        bcp = pltpu.make_async_copy(b_hbm, bbuf, psem.at[1])
        read(0, 0, 0, TB).start()
        gcp.start()
        bcp.start()

        def issue_read(i, c):
            read(i, i // CPS, (i % CPS) * TB, TB).start()
            return c
        jax.lax.fori_loop(1, NCU, issue_read, 0)
        last = [(NCU, M - TB, TB - TAIL), (NCU + 1, M - TAIL, TAIL)]
        for (i, off, n) in last:
            read(i, K - 1, off, n).start()
        gcp.wait()
        bcp.wait()

        def compute(s, off, n):
            def stage_a(j, c):
                s0 = pl.multiple_of(j * G, G)
                xf = xbuf[s, pl.ds(off + s0, G)].astype(jnp.float32)
                sc_ref[pl.ds(s0, G), :] = jnp.sum(xf * xf, axis=1)
                return c
            jax.lax.fori_loop(0, n // G, stage_a, 0)

            gf = gbuf[...].astype(jnp.float32).reshape(1, D)
            gx = jnp.sqrt(sc_ref[pl.ds(0, n), :])
            nx = gx / (jnp.mean(gx, axis=-1, keepdims=True) + 1e-6)
            sc_ref[pl.ds(0, n), :] = gf * nx + 1.0

            def stage_c(j, c):
                s0 = pl.multiple_of(j * G, G)
                bf = bbuf[...].astype(jnp.float32).reshape(1, 1, D)
                sc = sc_ref[pl.ds(s0, G), :]
                xf = xbuf[s, pl.ds(off + s0, G)].astype(jnp.float32)
                obuf[s, pl.ds(off + s0, G)] = (
                    xf * sc[:, None, :] + bf).astype(obuf.dtype)
                return c
            jax.lax.fori_loop(0, n // G, stage_c, 0)

        def issue_writes(lo, hi):
            def w(j, c):
                for h in range(_SPLIT):
                    pltpu.make_async_copy(
                        obuf.at[:, pl.ds(j, 1), pl.ds(h * SP, SP)],
                        o_hbm.at[:, pl.ds(j, 1), pl.ds(h * SP, SP)],
                        wsem.at[0]).start()
                return c
            jax.lax.fori_loop(lo, hi, w, 0)

        def main(i, c):
            s = i // CPS
            off = pl.multiple_of((i % CPS) * TB, TB)
            read(i, s, off, TB).wait()
            compute(s, off, TB)
            return c
        jax.lax.fori_loop(0, NCU, main, 0)

        (i0, off0, n0), (i1, off1, n1) = last
        read(i0, K - 1, off0, n0).wait()
        issue_writes(0, off0)
        compute(K - 1, off0, n0)
        issue_writes(off0, off1)
        read(i1, K - 1, off1, n1).wait()
        compute(K - 1, off1, n1)
        issue_writes(off1, M)
        pltpu.make_async_copy(obuf, o_hbm, wsem.at[0]).wait()

    out = pl.pallas_call(
        kernel_function,
        in_specs=[pl.BlockSpec(memory_space=pl.ANY)] * 3,
        out_specs=pl.BlockSpec(memory_space=pl.ANY),
        out_shape=jax.ShapeDtypeStruct((K, M, S, D), x.dtype),
        scratch_shapes=[
            pltpu.VMEM((K, M, S, D), x.dtype),
            pltpu.VMEM((K, M, S, D), x.dtype),
            pltpu.VMEM((D,), g.dtype),
            pltpu.VMEM((D,), b.dtype),
            pltpu.VMEM((TB, D), jnp.float32),
            pltpu.SemaphoreType.DMA((NCU + 2,)),
            pltpu.SemaphoreType.DMA((1,)),
            pltpu.SemaphoreType.DMA((2,)),
        ],
        compiler_params=pltpu.CompilerParams(vmem_limit_bytes=64 * 1024 * 1024),
    )(x.reshape(K, M, S, D), g, b)
    return out.reshape(B, S, D)
```

```python
import jax
import jax.numpy as jnp
import jax.experimental.pallas as pl
import jax.experimental.pallas.tpu as pltpu

_K = 8
_TB = 32
_HEAD = 16
_TAIL = 8
_G = 8
_SPLIT = 2


@jax.jit
def pallas_standalone__grn__sampling_kernel(
    x: jax.Array,
    g: jax.Array,
    b: jax.Array,
):
    B, S, D = x.shape
    K, TB, HEAD, TAIL, G = _K, _TB, _HEAD, _TAIL, _G
    M = B // K
    CPS = M // TB
    NCU = (K - 1) * CPS
    MID = M - HEAD - TAIL
    SP = S // _SPLIT
    assert B == K * M and M == CPS * TB and S == _SPLIT * SP
    assert all(n > 0 and n % G == 0 for n in (TB, HEAD, MID, TAIL))

    def kernel_function(x_hbm, g_hbm, b_hbm, o_hbm,
                        xbuf, obuf, gbuf, bbuf, sc_ref):

        def body(rsem, psem, wsem):
            def read(i, s, off, n):
                return pltpu.make_async_copy(
                    x_hbm.at[s, pl.ds(off, n)], xbuf.at[s, pl.ds(off, n)],
                    rsem.at[i])

            head = read(NCU, K - 1, 0, HEAD)
            mid = read(NCU + 1, K - 1, HEAD, MID)
            tail = read(NCU + 2, K - 1, HEAD + MID, TAIL)
            gcp = pltpu.make_async_copy(g_hbm, gbuf, psem.at[0])
            bcp = pltpu.make_async_copy(b_hbm, bbuf, psem.at[1])

            head.start()
            gcp.start()
            bcp.start()

            def issue_read(i, c):
                read(i, i // CPS, (i % CPS) * TB, TB).start()
                return c
            jax.lax.fori_loop(0, NCU, issue_read, 0)
            mid.start()
            tail.start()
            gcp.wait()
            bcp.wait()

            def compute(s, off, n):
                def stage_a(j, c):
                    s0 = pl.multiple_of(j * G, G)
                    xf = xbuf[s, pl.ds(off + s0, G)].astype(jnp.float32)
                    sc_ref[pl.ds(s0, G), :] = jnp.sum(xf * xf, axis=1)
                    return c
                jax.lax.fori_loop(0, n // G, stage_a, 0)

                gf = gbuf[...].astype(jnp.float32).reshape(1, D)
                gx = jnp.sqrt(sc_ref[pl.ds(0, n), :])
                nx = gx / (jnp.mean(gx, axis=-1, keepdims=True) + 1e-6)
                sc_ref[pl.ds(0, n), :] = gf * nx + 1.0

                def stage_c(j, c):
                    s0 = pl.multiple_of(j * G, G)
                    bf = bbuf[...].astype(jnp.float32).reshape(1, 1, D)
                    sc = sc_ref[pl.ds(s0, G), :]
                    xf = xbuf[s, pl.ds(off + s0, G)].astype(jnp.float32)
                    obuf[s, pl.ds(off + s0, G)] = (
                        xf * sc[:, None, :] + bf).astype(obuf.dtype)
                    return c
                jax.lax.fori_loop(0, n // G, stage_c, 0)

            def issue_writes(lo, hi):
                def wr(j, c):
                    for h in range(_SPLIT):
                        pltpu.make_async_copy(
                            obuf.at[:, pl.ds(j, 1), pl.ds(h * SP, SP)],
                            o_hbm.at[:, pl.ds(j, 1), pl.ds(h * SP, SP)],
                            wsem.at[0]).start()
                    return c
                jax.lax.fori_loop(lo, hi, wr, 0)

            head.wait()
            compute(K - 1, 0, HEAD)

            def main(i, c):
                s = i // CPS
                off = pl.multiple_of((i % CPS) * TB, TB)
                read(i, s, off, TB).wait()
                compute(s, off, TB)
                return c
            jax.lax.fori_loop(0, NCU, main, 0)

            mid.wait()
            issue_writes(0, HEAD)
            compute(K - 1, HEAD, MID)
            issue_writes(HEAD, HEAD + MID)
            tail.wait()
            compute(K - 1, HEAD + MID, TAIL)
            issue_writes(HEAD + MID, M)
            pltpu.make_async_copy(obuf, o_hbm, wsem.at[0]).wait()

        pl.run_scoped(
            body,
            pltpu.SemaphoreType.DMA((NCU + 3,)),
            pltpu.SemaphoreType.DMA((2,)),
            pltpu.SemaphoreType.DMA((1,)),
        )

    out = pl.pallas_call(
        kernel_function,
        in_specs=[pl.BlockSpec(memory_space=pl.ANY)] * 3,
        out_specs=pl.BlockSpec(memory_space=pl.ANY),
        out_shape=jax.ShapeDtypeStruct((K, M, S, D), x.dtype),
        scratch_shapes=[
            pltpu.VMEM((K, M, S, D), x.dtype),
            pltpu.VMEM((K, M, S, D), x.dtype),
            pltpu.VMEM((D,), g.dtype),
            pltpu.VMEM((D,), b.dtype),
            pltpu.VMEM((max(TB, HEAD, MID, TAIL), D), jnp.float32),
        ],
        compiler_params=pltpu.CompilerParams(
            vmem_limit_bytes=64 * 1024 * 1024),
    )(x.reshape(K, M, S, D), g, b)
    return out.reshape(B, S, D)
```

```python
import jax
import jax.numpy as jnp
import jax.experimental.pallas as pl
import jax.experimental.pallas.tpu as pltpu

_K = 8
_TB = 32
_HEAD = 16
_TAIL = 8
_G = 8
_SPLIT = 2


@jax.jit
def pallas_standalone__grn__sampling_kernel(
    x: jax.Array,
    g: jax.Array,
    b: jax.Array,
):
    B, S, D = x.shape
    K, TB, HEAD, TAIL, G = _K, _TB, _HEAD, _TAIL, _G
    M = B // K
    CPS = M // TB
    NCU = (K - 1) * CPS
    REST = M - HEAD
    MID = REST - TAIL
    SP = S // _SPLIT
    assert B == K * M and M == CPS * TB and S == _SPLIT * SP
    assert all(n > 0 and n % G == 0 for n in (TB, HEAD, REST))
    assert MID > 0 and TAIL > 0

    def kernel_function(x_hbm, g_hbm, b_hbm, o_hbm,
                        xbuf, obuf, gbuf, bbuf, sc_ref):

        def body(rsem, psem, wsem):
            def read(i, s, off, n):
                return pltpu.make_async_copy(
                    x_hbm.at[s, pl.ds(off, n)], xbuf.at[s, pl.ds(off, n)],
                    rsem.at[i])

            head = read(NCU, K - 1, 0, HEAD)
            mid = read(NCU + 1, K - 1, HEAD, MID)
            tail = read(NCU + 2, K - 1, HEAD + MID, TAIL)
            gcp = pltpu.make_async_copy(g_hbm, gbuf, psem.at[0])
            bcp = pltpu.make_async_copy(b_hbm, bbuf, psem.at[1])

            head.start()
            gcp.start()
            bcp.start()

            def issue_read(i, c):
                read(i, i // CPS, (i % CPS) * TB, TB).start()
                return c
            jax.lax.fori_loop(0, NCU, issue_read, 0)
            mid.start()
            tail.start()
            gcp.wait()
            bcp.wait()

            def compute(s, off, n):
                def stage_a(j, c):
                    s0 = pl.multiple_of(j * G, G)
                    xf = xbuf[s, pl.ds(off + s0, G)].astype(jnp.float32)
                    sc_ref[pl.ds(s0, G), :] = jnp.sum(xf * xf, axis=1)
                    return c
                jax.lax.fori_loop(0, n // G, stage_a, 0)

                gf = gbuf[...].astype(jnp.float32).reshape(1, D)
                gx = jnp.sqrt(sc_ref[pl.ds(0, n), :])
                nx = gx / (jnp.mean(gx, axis=-1, keepdims=True) + 1e-6)
                sc_ref[pl.ds(0, n), :] = gf * nx + 1.0

                def stage_c(j, c):
                    s0 = pl.multiple_of(j * G, G)
                    bf = bbuf[...].astype(jnp.float32).reshape(1, 1, D)
                    sc = sc_ref[pl.ds(s0, G), :]
                    xf = xbuf[s, pl.ds(off + s0, G)].astype(jnp.float32)
                    obuf[s, pl.ds(off + s0, G)] = (
                        xf * sc[:, None, :] + bf).astype(obuf.dtype)
                    return c
                jax.lax.fori_loop(0, n // G, stage_c, 0)

            def issue_writes(lo, hi):
                def wr(j, c):
                    for h in range(_SPLIT):
                        pltpu.make_async_copy(
                            obuf.at[:, pl.ds(j, 1), pl.ds(h * SP, SP)],
                            o_hbm.at[:, pl.ds(j, 1), pl.ds(h * SP, SP)],
                            wsem.at[0]).start()
                    return c
                jax.lax.fori_loop(lo, hi, wr, 0)

            head.wait()
            compute(K - 1, 0, HEAD)

            def main(i, c):
                s = i // CPS
                off = pl.multiple_of((i % CPS) * TB, TB)
                read(i, s, off, TB).wait()
                compute(s, off, TB)
                return c
            jax.lax.fori_loop(0, NCU, main, 0)

            mid.wait()
            issue_writes(0, HEAD)
            tail.wait()
            compute(K - 1, HEAD, REST)
            issue_writes(HEAD, M)
            pltpu.make_async_copy(obuf, o_hbm, wsem.at[0]).wait()

        pl.run_scoped(
            body,
            pltpu.SemaphoreType.DMA((NCU + 3,)),
            pltpu.SemaphoreType.DMA((2,)),
            pltpu.SemaphoreType.DMA((1,)),
        )

    out = pl.pallas_call(
        kernel_function,
        in_specs=[pl.BlockSpec(memory_space=pl.ANY)] * 3,
        out_specs=pl.BlockSpec(memory_space=pl.ANY),
        out_shape=jax.ShapeDtypeStruct((K, M, S, D), x.dtype),
        scratch_shapes=[
            pltpu.VMEM((K, M, S, D), x.dtype),
            pltpu.VMEM((K, M, S, D), x.dtype),
            pltpu.VMEM((D,), g.dtype),
            pltpu.VMEM((D,), b.dtype),
            pltpu.VMEM((max(TB, HEAD, REST), D), jnp.float32),
        ],
        compiler_params=pltpu.CompilerParams(
            vmem_limit_bytes=64 * 1024 * 1024),
    )(x.reshape(K, M, S, D), g, b)
    return out.reshape(B, S, D)
```
